```python
import jax
import jax.numpy as jnp

def _softmax(x, axis=-1):
    return jax.nn.softmax(x, axis=axis)
def _gelu(x):
    return jax.nn.gelu(x, approximate=True)
def _silu(x):
    return jax.nn.silu(x)
def _sigmoid(x):
    return jax.nn.sigmoid(x)
def _layernorm(x, axis=-1, eps=1e-5):
    m = jnp.mean(x, axis=axis, keepdims=True)
    v = jnp.var(x, axis=axis, keepdims=True)
    return (x - m) / jnp.sqrt(v + eps)
def _scatter_add(tgt, idx, src, axis=0):
    return tgt.at[idx].add(src)
def _segment_sum(src, seg, n):
    return jax.ops.segment_sum(src, seg, n)
class _Rng:
    def __init__(self, key):
        self._k = key
    def _next(self):
        self._k, sub = jax.random.split(self._k)
        return sub
    def normal(self, shape):
        return jax.random.normal(self._next(), shape, dtype=jnp.bfloat16)
    def randint(self, lo, hi, shape):
        return jax.random.randint(self._next(), shape, lo, hi, dtype=jnp.int32)
    def uniform(self, shape, lo=0.0, hi=1.0):
        return jax.random.uniform(self._next(), shape, jnp.bfloat16, lo, hi)
    def permutation(self, n):
        return jax.random.permutation(self._next(), n)


kernel_name = 'standalone__winograd__vision'

def setup_inputs():
    _rng = _Rng(jax.random.key(int.from_bytes(__import__("os").urandom(4), "little")))
    _w = (lambda a: (lambda t: t.astype(jnp.bfloat16) if jnp.issubdtype(t.dtype, jnp.floating) else t)(jnp.asarray(a)))
    H = W = 512 // 2 * 2
    C = 192
    return {
        "x": _w((lambda *s: _rng.normal(s) * 0.05)(1, H, W, C)),
        "w": _w((lambda *s: _rng.normal(s) * 0.05)(3, 3, C, C)),
    }

def reference(x, w):
    N, H, W, C = x.shape
    K = w.shape[-1]
    G  = jnp.array([[1.0,0.0,0.0],[0.5,0.5,0.5],[0.5,-0.5,0.5],[0.0,0.0,1.0]], dtype=x.dtype)
    Bt = jnp.array([[1.0,0.0,-1.0,0.0],[0.0,1.0,1.0,0.0],[0.0,-1.0,1.0,0.0],[0.0,1.0,0.0,-1.0]], dtype=x.dtype)
    At = jnp.array([[1.0,1.0,1.0,0.0],[0.0,1.0,-1.0,-1.0]], dtype=x.dtype)
    U = jnp.einsum("ar,rsck,bs->abck", G, w, G)
    xp = jnp.pad(x, ((0,0),(1,1),(1,1),(0,0)))
    nH, nW = H // 2, W // 2
    patches = []
    for i in range(4):
        for j in range(4):
            patches.append(xp[:, i:i + 2 * nH:2, j:j + 2 * nW:2, :])
    d = jnp.stack(patches).reshape(4, 4, N * nH * nW, C)
    V = jnp.einsum("ai,ijpc,bj->abpc", Bt, d, Bt)
    M = jnp.einsum("abck,abpc->abpk", U, V)
    Y = jnp.einsum("ma,abpk,nb->pmnk", At, M, At)
    Y = Y.reshape(N, nH, nW, 2, 2, K)
    Y = (lambda x, *d: x.transpose(*d))(Y, 0, 1, 3, 2, 4, 5).reshape(N, H, W, K)
    return Y
```

```python
import functools

import jax
import jax.numpy as jnp
import numpy as np
import jax.experimental.pallas as pl
import jax.experimental.pallas.tpu as pltpu

M_T = 6
N_T = M_T + 2
TILES = 2
W_CH = 512

_G = np.array([
    [1, 0, 0],
    [-2 / 9, -2 / 9, -2 / 9],
    [-2 / 9, 2 / 9, -2 / 9],
    [1 / 90, 1 / 45, 2 / 45],
    [1 / 90, -1 / 45, 2 / 45],
    [32 / 45, 16 / 45, 8 / 45],
    [32 / 45, -16 / 45, 8 / 45],
    [0, 0, 1]], dtype=np.float64)


def _in_tf(d):
    d0, d1, d2, d3, d4, d5, d6, d7 = d
    r0 = (d0 - d6) + 5.25 * (d4 - d2)
    r7 = (d7 - d1) + 5.25 * (d3 - d5)
    e = (d2 + d6) - 4.25 * d4
    o = (d1 + d5) - 4.25 * d3
    r1, r2 = e + o, e - o
    e = d6 + 0.25 * d2 - 1.25 * d4
    o = 0.5 * d1 - 2.5 * d3 + 2.0 * d5
    r3, r4 = e + o, e - o
    e = d6 + 4.0 * d2 - 5.0 * d4
    o = 2.0 * d1 - 2.5 * d3 + 0.5 * d5
    r5, r6 = e + o, e - o
    return [r0, r1, r2, r3, r4, r5, r6, r7]


def _out_tf(m):
    m0, m1, m2, m3, m4, m5, m6, m7 = m
    s1, t1 = m1 + m2, m1 - m2
    s2, t2 = m3 + m4, m3 - m4
    s3, t3 = m5 + m6, m5 - m6
    return [
        m0 + s1 + s2 + s3,
        t1 + 2.0 * t2 + 0.5 * t3,
        s1 + 4.0 * s2 + 0.25 * s3,
        t1 + 8.0 * t2 + 0.125 * t3,
        s1 + 16.0 * s2 + 0.0625 * s3,
        t1 + 32.0 * t2 + 0.03125 * t3 + m7,
    ]


def _kernel(x_hbm, w_ref, o_ref, xbuf, sem, u_ref, v_ref, m_ref, *, H, C, W):
    i = pl.program_id(0)
    nsteps = pl.num_programs(0)
    rows = M_T * TILES
    nin = rows + 2
    K = o_ref.shape[1]
    n_full_last = H - ((nsteps_static(H) - 1) * rows - 1)
    last = nsteps_static(H) - 1

    def copy_first(slot):
        return pltpu.make_async_copy(x_hbm.at[pl.ds(0, nin - 1)], xbuf.at[slot, pl.ds(1, nin - 1)], sem.at[slot])

    def copy_last(slot):
        return pltpu.make_async_copy(x_hbm.at[pl.ds(last * rows - 1, n_full_last)],
                                     xbuf.at[slot, pl.ds(0, n_full_last)], sem.at[slot])

    def copy_mid(step, slot):
        return pltpu.make_async_copy(x_hbm.at[pl.ds(step * rows - 1, nin)], xbuf.at[slot], sem.at[slot])

    slot = i % 2

    @pl.when(i == 0)
    def _():
        copy_first(0).start()
        xbuf[0, 0] = jnp.zeros((C, W), jnp.bfloat16)
        for s in range(3):
            ws = [w_ref[r, s].astype(jnp.float32) for r in range(3)]
            for a in range(N_T):
                acc = sum(float(_G[a, r]) * ws[r] for r in range(3) if _G[a, r] != 0)
                u_ref[a, :, s * C:(s + 1) * C] = acc.T.astype(jnp.bfloat16)

    @pl.when(i + 1 < last)
    def _():
        copy_mid(i + 1, 1 - slot).start()

    @pl.when(i + 1 == last)
    def _():
        copy_last(last % 2).start()
        for r in range(n_full_last, nin):
            xbuf[last % 2, r] = jnp.zeros((C, W), jnp.bfloat16)

    @pl.when(i == 0)
    def _():
        copy_first(0).wait()

    @pl.when(jnp.logical_and(i > 0, i < last))
    def _():
        copy_mid(i, slot).wait()

    @pl.when(i == last)
    def _():
        copy_last(last % 2).wait()

    lane = jax.lax.broadcasted_iota(jnp.int32, (8, W), 1)
    CH = 16

    def in_stage(t):
        for c0 in range(0, C, CH):
            d = [xbuf[slot, t * M_T + r, c0:c0 + CH, :].astype(jnp.float32) for r in range(N_T)]
            v = _in_tf(d)
            for a in range(N_T):
                vb = v[a].astype(jnp.bfloat16)
                vi = pltpu.bitcast(vb, jnp.int32)
                left = jnp.where(lane == 0, 0, pltpu.roll(vi, 1, 1))
                right = jnp.where(lane == W - 1, 0, pltpu.roll(vi, W - 1, 1))
                v_ref[t, a, c0:c0 + CH, :] = pltpu.bitcast(left, jnp.bfloat16)
                v_ref[t, a, C + c0:C + c0 + CH, :] = vb
                v_ref[t, a, 2 * C + c0:2 * C + c0 + CH, :] = pltpu.bitcast(right, jnp.bfloat16)

    def mm_stage(t):
        for a in range(N_T):
            m_ref[t, a] = jnp.dot(u_ref[a], v_ref[t, a], preferred_element_type=jnp.float32)

    def out_stage(t):
        for k0 in range(0, K, CH):
            y = _out_tf([m_ref[t, a, k0:k0 + CH, :] for a in range(N_T)])
            for r in range(M_T):
                o_ref[t * M_T + r, k0:k0 + CH, :] = y[r].astype(o_ref.dtype)

    for t in range(TILES):
        in_stage(t)
    for t in range(TILES):
        mm_stage(t)
    for t in range(TILES):
        out_stage(t)


def nsteps_static(H):
    return -(-H // (M_T * TILES))


@jax.jit
def pallas_standalone__winograd__vision_kernel(x: jax.Array, w: jax.Array):
    N, H, W, C = x.shape
    K = w.shape[-1]
    assert N == 1
    xt = x.transpose(0, 1, 3, 2).reshape(H, C, W)
    rows = M_T * TILES
    out = pl.pallas_call(
        functools.partial(_kernel, H=H, C=C, W=W),
        grid=(nsteps_static(H),),
        in_specs=[pl.BlockSpec(memory_space=pl.ANY), pl.BlockSpec(w.shape, lambda i: (0, 0, 0, 0))],
        out_specs=pl.BlockSpec((rows, K, W), lambda i: (i, 0, 0)),
        out_shape=jax.ShapeDtypeStruct((H, K, W), x.dtype),
        scratch_shapes=[
            pltpu.VMEM((2, rows + 2, C, W), jnp.bfloat16),
            pltpu.SemaphoreType.DMA((2,)),
            pltpu.VMEM((N_T, K, 3 * C), jnp.bfloat16),
            pltpu.VMEM((TILES, N_T, 3 * C, W), jnp.bfloat16),
            pltpu.VMEM((TILES, N_T, K, W), jnp.float32),
        ],
        compiler_params=pltpu.CompilerParams(
            dimension_semantics=("arbitrary",), vmem_limit_bytes=100 * 2**20),
    )(xt, w)
    return out.reshape(1, H, K, W).transpose(0, 1, 3, 2)
```

```python
import functools

import jax
import jax.numpy as jnp
import numpy as np
import jax.experimental.pallas as pl
import jax.experimental.pallas.tpu as pltpu

TILES = 8
ROWS = 4 * TILES
CH = 16

_P, _Q = 1.5, 2.0 / 3.0
_N = [_P * _P * _Q * _Q, -2 * _P * _P * (_P * _P - _Q * _Q), 2 * _Q * _Q * (_P * _P - _Q * _Q)]
_G = np.array([
    [1 / _N[0], 0, 0],
    [-1 / _N[1], -_P / _N[1], -_P * _P / _N[1]],
    [-1 / _N[1], _P / _N[1], -_P * _P / _N[1]],
    [-1 / _N[2], -_Q / _N[2], -_Q * _Q / _N[2]],
    [-1 / _N[2], _Q / _N[2], -_Q * _Q / _N[2]],
    [0, 0, 1]], dtype=np.float64)


def _in_tf(d):
    d0, d1, d2, d3, d4, d5 = d
    c = _P * _P + _Q * _Q
    r0 = (d0 + d4) - c * d2
    r5 = (d1 + d5) - c * d3
    e = d4 - (_Q * _Q) * d2
    o = _P * d3 - _Q * d1
    r1, r2 = e + o, e - o
    e = d4 - (_P * _P) * d2
    o = _Q * d3 - _P * d1
    r3, r4 = e + o, e - o
    return [r0, r1, r2, r3, r4, r5]


def _out_tf(m):
    m0, m1, m2, m3, m4, m5 = m
    s1, t1 = m1 + m2, m1 - m2
    s2, t2 = m3 + m4, m3 - m4
    return [
        m0 + s1 + s2,
        _P * t1 + _Q * t2,
        (_P * _P) * s1 + (_Q * _Q) * s2,
        (_P ** 3) * t1 + (_Q ** 3) * t2 + m5,
    ]


def _kernel(x_hbm, x0_ref, w_ref, o_ref, xbuf, sem, u_ref, z_ref, v_ref, m_ref, *, H, C, W):
    i = pl.program_id(0)
    K = o_ref.shape[1]
    last = H // ROWS - 1
    slot = i % 2
    f32, bf16, i32 = jnp.float32, jnp.bfloat16, jnp.int32

    def copy(step, sl):
        return pltpu.make_async_copy(x_hbm.at[pl.ds(step * ROWS + 1, ROWS)], xbuf.at[sl], sem.at[sl])

    def copy_last():
        return pltpu.make_async_copy(x_hbm.at[pl.ds(last * ROWS + 1, ROWS - 1)],
                                     xbuf.at[last % 2, pl.ds(0, ROWS - 1)], sem.at[last % 2])

    lane = jax.lax.broadcasted_iota(i32, (CH // 2, 128), 1)
    grp = lane // 32
    j32 = lane % 32
    gidx = [4 * j32 + (grp - q) % 4 for q in range(4)]
    oidx = [((lane % 4 + q) % 4) * 32 + lane // 4 for q in range(4)]
    odd = (grp % 2) == 1
    hi = grp >= 2
    hi1 = ((grp + 3) % 4) >= 2

    def shuffle4(a):
        b0 = jnp.where(odd, a[1], a[0])
        b1 = jnp.where(odd, a[0], a[1])
        b2 = jnp.where(odd, a[3], a[2])
        b3 = jnp.where(odd, a[2], a[3])
        return [jnp.where(hi, b2, b0), jnp.where(hi1, b3, b1),
                jnp.where(hi, b0, b2), jnp.where(hi1, b1, b3)]

    def w_stage(load, zrow):
        for c0 in range(0, C, CH):
            xi = pltpu.bitcast(load(c0), i32)
            a = [jnp.take_along_axis(xi[:, q * 128:(q + 1) * 128], gidx[q], axis=1) for q in range(4)]
            s = shuffle4(a)
            ph = [s[0]] + [pltpu.roll(s[p], 128 - 32 * p, 1) for p in (1, 2, 3)]
            dm = jnp.where(lane == 0, 0, pltpu.roll(s[3], 33, 1))
            dp = jnp.where(lane == 127, 0, pltpu.roll(s[0], 127, 1))
            src = [dm] + ph + [dp]
            for h in range(2):
                d = [pltpu.bitcast(t << 16 if h == 0 else t & np.int32(-65536), f32) for t in src]
                z = _in_tf(d)
                for b in range(6):
                    z_ref[zrow, b, c0 + 8 * h:c0 + 8 * h + 8, :] = z[b]

    @pl.when(i == 0)
    def _():
        copy(0, 0).start()
        for a in range(6):
            t = [sum(float(_G[a, r]) * w_ref[r, s].astype(f32) for r in range(3) if _G[a, r] != 0)
                 for s in range(3)]
            for b in range(6):
                acc = sum(float(_G[b, s]) * t[s] for s in range(3) if _G[b, s] != 0)
                u_ref[a, b] = pltpu.bitcast(acc.T.astype(bf16), i32)
        z_ref[0] = jnp.zeros(z_ref.shape[1:], f32)
        w_stage(lambda c0: x0_ref[0, c0:c0 + CH, :], 1)

    @pl.when(i > 0)
    def _():
        z_ref[0] = z_ref[ROWS]
        z_ref[1] = z_ref[ROWS + 1]

    @pl.when(i + 1 < last)
    def _():
        copy(i + 1, 1 - slot).start()

    @pl.when(i + 1 == last)
    def _():
        copy_last().start()
        xbuf[last % 2, ROWS - 1] = jnp.zeros((C, W), bf16)

    @pl.when(i < last)
    def _():
        copy(i, slot).wait()

    @pl.when(i == last)
    def _():
        copy_last().wait()

    def pack(lo, hi_):
        return pltpu.bitcast(pltpu.pack_elementwise([lo, hi_], packed_dtype=bf16), i32)

    def h_stage(t):
        for b in range(6):
            for c0 in range(0, C, CH):
                v = [_in_tf([z_ref[4 * t + r, b, c0 + 8 * h:c0 + 8 * h + 8, :] for r in range(6)])
                     for h in range(2)]
                for a in range(6):
                    v_ref[t, a, b, c0 // 2:(c0 + CH) // 2, :] = pack(v[0][a], v[1][a])

    def mm_stage(t):
        for b in range(6):
            for a in range(6):
                m_ref[t, a, b] = jnp.dot(pltpu.bitcast(u_ref[a, b], bf16), pltpu.bitcast(v_ref[t, a, b], bf16), preferred_element_type=f32)

    def out_stage(t):
        for k0 in range(0, K, CH):
            ys = []
            for h in range(2):
                cols = [_out_tf([m_ref[t, a, b, pl.ds(k0 + h, 8, stride=2), :] for a in range(6)])
                        for b in range(6)]
                ys.append([_out_tf([cols[b][r] for b in range(6)]) for r in range(4)])
            for r in range(4):
                y = [ys[0][r], ys[1][r]]
                y = [pack(y[0][p], y[1][p]) for p in range(4)]
                y = [y[0]] + [pltpu.roll(y[p], 32 * p, 1) for p in (1, 2, 3)]
                s = shuffle4(y)
                for q in range(4):
                    o = jnp.take_along_axis(s[q], oidx[q], axis=1)
                    o_ref[4 * t + r, k0:k0 + CH, q * 128:(q + 1) * 128] = pltpu.bitcast(o, bf16)

    for t in range(TILES):
        for r in range(4):
            row = 4 * t + r
            w_stage(lambda c0, row=row: xbuf[slot, row, c0:c0 + CH, :], row + 2)
        h_stage(t)
        mm_stage(t)
        out_stage(t)


@jax.jit
def pallas_standalone__winograd__vision_kernel(x: jax.Array, w: jax.Array):
    N, H, W, C = x.shape
    K = w.shape[-1]
    assert N == 1 and W == 512 and H % ROWS == 0
    xt = x.transpose(0, 1, 3, 2).reshape(H, C, W)
    out = pl.pallas_call(
        functools.partial(_kernel, H=H, C=C, W=W),
        grid=(H // ROWS,),
        in_specs=[pl.BlockSpec(memory_space=pl.ANY),
                  pl.BlockSpec((1, C, W), lambda i: (0, 0, 0)),
                  pl.BlockSpec(w.shape, lambda i: (0, 0, 0, 0))],
        out_specs=pl.BlockSpec((ROWS, K, W), lambda i: (i, 0, 0)),
        out_shape=jax.ShapeDtypeStruct((H, K, W), x.dtype),
        scratch_shapes=[
            pltpu.VMEM((2, ROWS, C, W), jnp.bfloat16),
            pltpu.SemaphoreType.DMA((2,)),
            pltpu.VMEM((6, 6, K // 2, C), jnp.int32),
            pltpu.VMEM((ROWS + 2, 6, C, 128), jnp.float32),
            pltpu.VMEM((TILES, 6, 6, C // 2, 128), jnp.int32),
            pltpu.VMEM((TILES, 6, 6, K, 128), jnp.float32),
        ],
        compiler_params=pltpu.CompilerParams(
            dimension_semantics=("arbitrary",), vmem_limit_bytes=120 * 2**20),
    )(xt, xt, w)
    return out.reshape(1, H, K, W).transpose(0, 1, 3, 2)
```
